```python
import jax
import jax.numpy as jnp

def _softmax(x, axis=-1):
    return jax.nn.softmax(x, axis=axis)
def _gelu(x):
    return jax.nn.gelu(x, approximate=True)
def _silu(x):
    return jax.nn.silu(x)
def _sigmoid(x):
    return jax.nn.sigmoid(x)
def _layernorm(x, axis=-1, eps=1e-5):
    m = jnp.mean(x, axis=axis, keepdims=True)
    v = jnp.var(x, axis=axis, keepdims=True)
    return (x - m) / jnp.sqrt(v + eps)
def _scatter_add(tgt, idx, src, axis=0):
    return tgt.at[idx].add(src)
def _segment_sum(src, seg, n):
    return jax.ops.segment_sum(src, seg, n)
class _Rng:
    def __init__(self, key):
        self._k = key
    def _next(self):
        self._k, sub = jax.random.split(self._k)
        return sub
    def normal(self, shape):
        return jax.random.normal(self._next(), shape, dtype=jnp.bfloat16)
    def randint(self, lo, hi, shape):
        return jax.random.randint(self._next(), shape, lo, hi, dtype=jnp.int32)
    def uniform(self, shape, lo=0.0, hi=1.0):
        return jax.random.uniform(self._next(), shape, jnp.bfloat16, lo, hi)
    def permutation(self, n):
        return jax.random.permutation(self._next(), n)


kernel_name = 'parallel_sum__sliding_block_cached__mixer_s_mlp__decode'

def setup_inputs():
    _rng = _Rng(jax.random.key(int.from_bytes(__import__("os").urandom(4), "little")))
    _w = (lambda a: (lambda t: t.astype(jnp.bfloat16) if jnp.issubdtype(t.dtype, jnp.floating) else t)(jnp.asarray(a)))
    def _A_setup():
        B, Sq, D = 4, 1, 512
        Hq, Hkv, Sk, Dh = 32, 32, 8192, 128
        assert Hq % Hkv == 0, (Hq, Hkv)
        return {
            "x": _w((lambda *s: _rng.normal(s) * 0.05)(B, Sq, D)),
            "k_cache": _w((lambda *s: _rng.normal(s) * 0.05)(B, Hkv, Sk, Dh)),
            "v_cache": _w((lambda *s: _rng.normal(s) * 0.05)(B, Hkv, Sk, Dh)),
            "wq": _w((lambda *s: _rng.normal(s) * 0.05)(D, Hq * Dh) * (D ** -0.5)),
            "wo": _w((lambda *s: _rng.normal(s) * 0.05)(Hq * Dh, D) * ((Hq * Dh) ** -0.5)),
        }
    _A_in = _A_setup()

    def _B_setup():
        B, S, D, F = 4, 1, 512, 1376
        return {
            "x":  _w((lambda *s: _rng.normal(s) * 0.05)(B, S, D)),
            "w1": _w((lambda *s: _rng.normal(s) * 0.05)(D, D) * (D ** -0.5)),
            "w2": _w((lambda *s: _rng.normal(s) * 0.05)(D, D) * (D ** -0.5)),
            "w3": _w((lambda *s: _rng.normal(s) * 0.05)(D, F) * (D ** -0.5)),
            "w4": _w((lambda *s: _rng.normal(s) * 0.05)(F, D) * (F ** -0.5)),
        }
    _B_in = _B_setup()

    return {
        "A_x": _A_in["x"],
        "A_k_cache": _A_in["k_cache"],
        "A_v_cache": _A_in["v_cache"],
        "A_wq": _A_in["wq"],
        "A_wo": _A_in["wo"],
        "B_x": _B_in["x"],
        "B_w1": _B_in["w1"],
        "B_w2": _B_in["w2"],
        "B_w3": _B_in["w3"],
        "B_w4": _B_in["w4"],
    }

def reference(A_x, A_k_cache, A_v_cache, A_wq, A_wo, B_x, B_w1, B_w2, B_w3, B_w4):
    def _A_ref(x, k_cache, v_cache, wq, wo):
        B, Sq, D = x.shape
        Hq, Dh = 32, 128
        Hkv, Sk = k_cache.shape[1], k_cache.shape[2]
        W = min(4096, max(256, Sk // 4))
        rep = Hq // Hkv
        q = (lambda x, *d: x.transpose(*d))((x @ wq).reshape(B, Sq, Hq, Dh), 0, 2, 1, 3)
        k = jnp.repeat(k_cache[:, :, Sk - W:, :], rep, axis=1)
        v = jnp.repeat(v_cache[:, :, Sk - W:, :], rep, axis=1)
        scores = jnp.einsum("bhqd,bhkd->bhqk", q, k) * (Dh ** -0.5)
        p = _softmax(scores, axis=-1)
        o = jnp.einsum("bhqk,bhkd->bhqd", p, v)
        return (lambda x, *d: x.transpose(*d))(o, 0, 2, 1, 3).reshape(B, Sq, Hq * Dh) @ wo

    def _B_ref(x, w1, w2, w3, w4):
        B, S, D = x.shape
        h = _gelu(_layernorm(x, axis=-1) @ w1)
        c = D // 4
        g0 = jnp.pad(h[:, :, 0*c:1*c], ((0, 0), (1, 0), (0, 0)))[:, :S, :]
        g1 = jnp.pad(h[:, :, 1*c:2*c], ((0, 0), (0, 1), (0, 0)))[:, 1:, :]
        g2 = jnp.pad(h[:, :, 2*c:3*c], ((0, 0), (2, 0), (0, 0)))[:, :S, :]
        g3 = jnp.pad(h[:, :, 3*c:   ], ((0, 0), (0, 2), (0, 0)))[:, 2:, :]
        hs = jnp.concatenate([g0, g1, g2, g3], axis=-1) @ w2
        x1 = x + hs
        h2 = _gelu(_layernorm(x1, axis=-1) @ w3) @ w4
        return x1 + h2

    x = A_x
    xn = _layernorm(x, axis=-1)
    return x + _A_ref(xn, A_k_cache, A_v_cache, A_wq, A_wo) + _B_ref(xn, B_w1, B_w2, B_w3, B_w4)
```

```python
import jax
import jax.numpy as jnp
from jax import lax
import jax.experimental.pallas as pl
import jax.experimental.pallas.tpu as pltpu

_NT = (((1,), (1,)), ((), ()))


def _layernorm(x, eps=1e-5):
    m = jnp.mean(x, axis=-1, keepdims=True)
    d = x - m
    v = jnp.mean(d * d, axis=-1, keepdims=True)
    return d / jnp.sqrt(v + eps)


def make(nslots=4, two_queues=True, w4_pieces=(512, 512, 256, 96), bounds_checks=False):
    def fn(A_x, A_k_cache, A_v_cache, A_wq, A_wo, B_x, B_w1, B_w2, B_w3, B_w4):
        B, Sq, D = A_x.shape
        _, H, Sk, Dh = A_k_cache.shape
        F = B_w3.shape[1]
        W = min(4096, max(256, Sk // 4))
        W0 = Sk - W
        scale = Dh ** -0.5
        f32, bf16 = jnp.float32, jnp.bfloat16
        assert sum(w4_pieces) == F
        w4_offs = [sum(w4_pieces[:i]) for i in range(len(w4_pieces))]

        def kernel(x_hbm, k_hbm, v_hbm, wq_hbm, wo_hbm, w3t_hbm, w4_hbm, o_ref,
                   x_vm, wq_vm, wo_vm, w3_vm, w4_vm, kbuf, vbuf, q_vm,
                   wsem, ksem, vsem, w4sem):
            def prio(i):
                return (i % 2) if two_queues else 0

            def kcp(h, b, slot):
                return pltpu.make_async_copy(
                    k_hbm.at[b, h, pl.ds(W0, W), :], kbuf.at[slot, b], ksem.at[slot, b])

            def vcp(h, b, slot):
                return pltpu.make_async_copy(
                    v_hbm.at[b, h, pl.ds(W0, W), :], vbuf.at[slot, b], vsem.at[slot, b])

            def start_head(h, slot):
                for b in range(B):
                    kcp(h, b, slot).start(priority=prio(b))
                for b in range(B):
                    vcp(h, b, slot).start(priority=prio(b))

            hd = D // 2
            xcp = pltpu.make_async_copy(x_hbm, x_vm, wsem.at[0])
            wqcp = [pltpu.make_async_copy(wq_hbm.at[pl.ds(i * hd, hd)], wq_vm.at[pl.ds(i * hd, hd)], wsem.at[1 + i]) for i in range(2)]
            ho = H * Dh // 2
            wocp = [pltpu.make_async_copy(wo_hbm.at[pl.ds(i * ho, ho)], wo_vm.at[pl.ds(i * ho, ho)], wsem.at[3 + i]) for i in range(2)]
            hf = F // 2
            w3cp = [pltpu.make_async_copy(w3t_hbm.at[pl.ds(i * hf, hf)], w3_vm.at[pl.ds(i * hf, hf)], wsem.at[5 + i]) for i in range(2)]
            w4cp = [pltpu.make_async_copy(w4_hbm.at[pl.ds(o, n)], w4_vm.at[pl.ds(o, n)], w4sem.at[i])
                    for i, (o, n) in enumerate(zip(w4_offs, w4_pieces))]

            xcp.start()
            for i in range(2):
                wqcp[i].start(priority=prio(i))
            for i in range(2):
                w3cp[i].start(priority=prio(i))
            for i in range(2):
                wocp[i].start(priority=prio(i))
            for s in range(nslots):
                start_head(s, s)

            xcp.wait()
            x = x_vm[...].astype(f32)
            xn = _layernorm(x).astype(bf16)
            xn2 = _layernorm(xn.astype(f32)).astype(bf16)
            for c in wqcp:
                c.wait()
            for h in range(H):
                q = jnp.dot(xn, wq_vm[:, h * Dh:(h + 1) * Dh], preferred_element_type=f32)
                q_vm[h] = q
            for c in w3cp:
                c.wait()
            g = lax.dot_general(xn2, w3_vm[...], _NT, preferred_element_type=f32)
            g = jax.nn.gelu(g, approximate=True).astype(bf16)
            for c in wocp:
                c.wait()

            row_s = lax.broadcasted_iota(jnp.int32, (B, W), 0)
            row_o = lax.broadcasted_iota(jnp.int32, (B, Dh), 0)

            def head(h, acc):
                slot = lax.rem(h, nslots)
                q = q_vm[h].astype(bf16)
                s = None
                for b in range(B):
                    kcp(h, b, slot).wait()
                    sb = lax.dot_general(q, kbuf[slot, b], _NT, preferred_element_type=f32)
                    s = sb if s is None else jnp.where(row_s == b, sb, s)
                s = s * scale
                m = jnp.max(s, axis=-1, keepdims=True)
                p = jnp.exp(s - m)
                l = jnp.sum(p, axis=-1, keepdims=True)
                pb = p.astype(bf16)
                o = None
                for b in range(B):
                    vcp(h, b, slot).wait()
                    ob = jnp.dot(pb, vbuf[slot, b], preferred_element_type=f32)
                    o = ob if o is None else jnp.where(row_o == b, ob, o)
                o = (o / l).astype(bf16)

                @pl.when(h + nslots < H)
                def _():
                    start_head(h + nslots, slot)

                @pl.when(h + nslots == H)
                def _():
                    for i, c in enumerate(w4cp):
                        c.start(priority=prio(i))

                r0 = pl.multiple_of(h * Dh, Dh)
                return acc + jnp.dot(o, wo_vm[pl.ds(r0, Dh), :], preferred_element_type=f32)

            acc = lax.fori_loop(0, H, head, x + xn.astype(f32))
            for c, o, n in zip(w4cp, w4_offs, w4_pieces):
                c.wait()
                acc = acc + jnp.dot(g[:, o:o + n], w4_vm[pl.ds(o, n), :], preferred_element_type=f32)
            o_ref[...] = acc.astype(o_ref.dtype)

        out = pl.pallas_call(
            kernel,
            in_specs=[pl.BlockSpec(memory_space=pltpu.HBM)] * 7,
            out_specs=pl.BlockSpec(memory_space=pltpu.VMEM),
            out_shape=jax.ShapeDtypeStruct((B, D), A_x.dtype),
            scratch_shapes=[
                pltpu.VMEM((B, D), bf16),
                pltpu.VMEM((D, H * Dh), bf16),
                pltpu.VMEM((H * Dh, D), bf16),
                pltpu.VMEM((F, D), bf16),
                pltpu.VMEM((F, D), bf16),
                pltpu.VMEM((nslots, B, W, Dh), bf16),
                pltpu.VMEM((nslots, B, W, Dh), bf16),
                pltpu.VMEM((H, B, Dh), f32),
                pltpu.SemaphoreType.DMA((7,)),
                pltpu.SemaphoreType.DMA((nslots, B)),
                pltpu.SemaphoreType.DMA((nslots, B)),
                pltpu.SemaphoreType.DMA((len(w4_pieces),)),
            ],
            compiler_params=pltpu.CompilerParams(
                vmem_limit_bytes=100 * 1024 * 1024,
                disable_bounds_checks=not bounds_checks),
        )(A_x.reshape(B, D), A_k_cache, A_v_cache, A_wq, A_wo, B_w3.T, B_w4)
        return out.reshape(B, Sq, D)
    return fn


_impl = make(nslots=2)


@jax.jit
def pallas_parallel_sum__sliding_block_cached__mixer_s_mlp__decode_kernel(
    A_x, A_k_cache, A_v_cache, A_wq, A_wo, B_x, B_w1, B_w2, B_w3, B_w4
):
    return _impl(A_x, A_k_cache, A_v_cache, A_wq, A_wo, B_x, B_w1, B_w2, B_w3, B_w4)
```

```python
import jax
import jax.numpy as jnp
from jax import lax
import jax.experimental.pallas as pl
import jax.experimental.pallas.tpu as pltpu

_NT = (((1,), (1,)), ((), ()))


def _layernorm(x, eps=1e-5):
    m = jnp.mean(x, axis=-1, keepdims=True)
    d = x - m
    v = jnp.mean(d * d, axis=-1, keepdims=True)
    return d / jnp.sqrt(v + eps)


def make(nslots=2, R=32, NS=4, wo_groups=(512, 256, 128, 64, 32, 32), unroll=4, sem_checks=False,
         compute=True):
    def fn(A_x, A_k_cache, A_v_cache, A_wq, A_wo, B_x, B_w1, B_w2, B_w3, B_w4):
        B, Sq, D = A_x.shape
        _, H, Sk, Dh = A_k_cache.shape
        F = B_w3.shape[1]
        W = min(4096, max(256, Sk // 4))
        W0 = Sk - W
        HD = H * Dh
        scale = Dh ** -0.5
        f32, bf16 = jnp.float32, jnp.bfloat16
        NP = W // R
        OR = HD // NS
        RO = 32 // NS
        assert sum(wo_groups) == OR
        wo_offs = [sum(wo_groups[:i]) for i in range(len(wo_groups))]

        def kernel(x_hbm, k_hbm, v_hbm, wq_hbm, wo_hbm, w3t_hbm, w4_hbm, o_ref,
                   x_vm, wq_vm, wo_vm, w3_vm, w4_vm, kv, q_vm, p_vm, a_vm,
                   wsem, kvsem, wosem):

            def loop(n, body, unroll=unroll):
                lax.fori_loop(0, n, lambda i, _: body(i), None, unroll=unroll)

            def kv_piece(which, h, slot, i):
                r = pl.multiple_of(i * R, R)
                return pltpu.make_async_copy(
                    (k_hbm, v_hbm)[which].at[:, h, pl.ds(W0 + r, R), :],
                    kv.at[slot, which, :, pl.ds(r, R), :], kvsem.at[slot, which])

            def kv_wait(which, slot):
                pltpu.make_async_copy(kv.at[slot, which], kv.at[slot, which], kvsem.at[slot, which]).wait()

            def rows_piece(src, dst, sem, i):
                r = pl.multiple_of(i * 32, 32)
                return pltpu.make_async_copy(src.at[pl.ds(r, 32), :], dst.at[pl.ds(r, 32), :], sem)

            def wq_piece(i, j):
                r = pl.multiple_of(i * 8, 8)
                c = pl.ds(j * (HD // 2), HD // 2)
                return pltpu.make_async_copy(wq_hbm.at[pl.ds(r, 8), c], wq_vm.at[pl.ds(r, 8), c], wsem.at[1])

            def wo_piece(g, i):
                r = pl.multiple_of(wo_offs[g] + i * RO, RO)
                return pltpu.make_async_copy(wo_hbm.at[:, pl.ds(r, RO), :], wo_vm.at[:, pl.ds(r, RO), :], wosem.at[g])

            def wait_all(ref, sem):
                pltpu.make_async_copy(ref, ref, sem).wait()

            def issue_step(t, slot, lo, n):
                def body(i):
                    kv_piece(0, t + 1, slot, lo + i).start(priority=0)
                    kv_piece(1, t, slot, lo + i).start(priority=1)
                loop(n, body)

            row_s = lax.broadcasted_iota(jnp.int32, (B, W), 0)
            row_o = lax.broadcasted_iota(jnp.int32, (B, Dh), 0)

            def probs(h, slot):
                q = q_vm[h].astype(bf16)
                s = None
                for b in range(B):
                    sb = lax.dot_general(q, kv[slot, 0, b], _NT, preferred_element_type=f32)
                    s = sb if s is None else jnp.where(row_s == b, sb, s)
                s = s * scale
                m = jnp.max(s, axis=-1, keepdims=True)
                p = jnp.exp(s - m)
                return p, jnp.sum(p, axis=-1, keepdims=True)

            def attend(p, l, slot):
                pb = p.astype(bf16)
                o = None
                for b in range(B):
                    ob = jnp.dot(pb, kv[slot, 1, b], preferred_element_type=f32)
                    o = ob if o is None else jnp.where(row_o == b, ob, o)
                return o / l

            xcp = pltpu.make_async_copy(x_hbm, x_vm, wsem.at[0])
            xcp.start()
            last = nslots - 1
            nf = F // 32
            assert D // 8 == NP

            def phase_a1(i):
                wq_piece(i, 0).start(priority=0)
                kv_piece(0, 0, last, i).start(priority=1)
                wq_piece(lax.rem(i + NP // 2, NP), 1).start(priority=0)
                rows_piece(w3t_hbm, w3_vm, wsem.at[2], i).start(priority=1)
            loop(nf, phase_a1, unroll=1)

            def phase_a2(j):
                for u in range(2):
                    i = nf + 2 * j + u
                    wq_piece(i, 0).start(priority=u)
                    kv_piece(0, 0, last, i).start(priority=1 - u)
                    wq_piece(lax.rem(i + NP // 2, NP), 1).start(priority=u)
            loop((NP - nf) // 2, phase_a2, unroll=1)
            if (NP - nf) % 2:
                i = NP - 1
                wq_piece(i, 0).start(priority=0)
                kv_piece(0, 0, last, i).start(priority=1)
                wq_piece((i + NP // 2) % NP, 1).start(priority=0)

            issue_step(0, 0, 0, NP // 2)
            xcp.wait()
            x = x_vm[...].astype(f32)
            xn = _layernorm(x).astype(bf16)
            xn2 = _layernorm(xn.astype(f32)).astype(bf16)
            wait_all(wq_vm, wsem.at[1])
            if compute:
                for h in range(H):
                    q_vm[h] = jnp.dot(xn, wq_vm[:, h * Dh:(h + 1) * Dh], preferred_element_type=f32)
            issue_step(0, 0, NP // 2, NP // 2)
            wait_all(w3_vm, wsem.at[2])
            kv_wait(0, last)
            if compute:
                g = lax.dot_general(xn2, w3_vm[...], _NT, preferred_element_type=f32)
                g = jax.nn.gelu(g, approximate=True).astype(bf16)
                p0, l0 = probs(0, last)
                p_vm[...] = p0
            else:
                l0 = jnp.zeros((B, 1), f32)

            def step(t, l):
                slot = lax.rem(t, nslots)
                nxt = lax.rem(t + 1, nslots)

                @pl.when(t < H - 2)
                def _():
                    issue_step(t + 1, nxt, 0, NP)

                @pl.when(t == H - 2)
                def _():
                    def body1(i):
                        rows_piece(w4_hbm, w4_vm, wsem.at[3], i).start(priority=0)
                        kv_piece(1, H - 1, nxt, i).start(priority=1)
                    loop(nf, body1, unroll=1)
                    for i in range(nf, NP):
                        kv_piece(1, H - 1, nxt, i).start(priority=i % 2)

                kv_wait(0, slot)
                kv_wait(1, slot)
                if not compute:
                    return l
                a_vm[t] = attend(p_vm[...], l, slot)
                p, l = probs(t + 1, slot)
                p_vm[...] = p
                return l

            l = lax.fori_loop(0, H - 1, step, l0)

            def issue_wo(g):
                n = wo_groups[g] // RO

                def body(i):
                    wo_piece(g, i).start(priority=0)
                    wo_piece(g, i + n // 2).start(priority=1)
                loop(n // 2, body, unroll=min(unroll, n // 2))

            issue_wo(0)
            slot = (H - 1) % nslots
            kv_wait(1, slot)
            wait_all(w4_vm, wsem.at[3])
            acc = x + xn.astype(f32)
            if compute:
                a_vm[H - 1] = attend(p_vm[...], l, slot)
                acc = acc + jnp.dot(g, w4_vm[...], preferred_element_type=f32)
            for gi in range(1, len(wo_groups)):
                issue_wo(gi)
            for gi, (o, n) in enumerate(zip(wo_offs, wo_groups)):
                wait_all(wo_vm.at[:, pl.ds(o, n), :], wosem.at[gi])
                if not compute:
                    continue
                for j in range(NS):
                    if n >= Dh:
                        h0 = (j * OR + o) // Dh
                        a = jnp.concatenate([a_vm[h0 + u] for u in range(n // Dh)], axis=-1)
                    else:
                        h0, c0 = divmod(j * OR + o, Dh)
                        a = a_vm[h0][:, c0:c0 + n]
                    acc = acc + jnp.dot(a.astype(bf16), wo_vm[j, pl.ds(o, n), :], preferred_element_type=f32)
            o_ref[...] = acc.astype(o_ref.dtype)

        out = pl.pallas_call(
            kernel,
            in_specs=[pl.BlockSpec(memory_space=pltpu.HBM)] * 7,
            out_specs=pl.BlockSpec(memory_space=pltpu.VMEM),
            out_shape=jax.ShapeDtypeStruct((B, D), A_x.dtype),
            scratch_shapes=[
                pltpu.VMEM((B, D), bf16),
                pltpu.VMEM((D, HD), bf16),
                pltpu.VMEM((NS, OR, D), bf16),
                pltpu.VMEM((F, D), bf16),
                pltpu.VMEM((F, D), bf16),
                pltpu.VMEM((nslots, 2, B, W, Dh), bf16),
                pltpu.VMEM((H, B, Dh), f32),
                pltpu.VMEM((B, W), f32),
                pltpu.VMEM((H, B, Dh), f32),
                pltpu.SemaphoreType.DMA((4,)),
                pltpu.SemaphoreType.DMA((nslots, 2)),
                pltpu.SemaphoreType.DMA((len(wo_groups),)),
            ],
            compiler_params=pltpu.CompilerParams(
                vmem_limit_bytes=100 * 1024 * 1024,
                disable_bounds_checks=True,
                disable_semaphore_checks=not sem_checks),
        )(A_x.reshape(B, D), A_k_cache, A_v_cache, A_wq, A_wo.reshape(NS, OR, D), B_w3.T, B_w4)
        return out.reshape(B, Sq, D)
    return fn


_impl = make(wo_groups=(512, 384, 128))


@jax.jit
def pallas_parallel_sum__sliding_block_cached__mixer_s_mlp__decode_kernel(
    A_x, A_k_cache, A_v_cache, A_wq, A_wo, B_x, B_w1, B_w2, B_w3, B_w4
):
    return _impl(A_x, A_k_cache, A_v_cache, A_wq, A_wo, B_x, B_w1, B_w2, B_w3, B_w4)
```

```python
import jax
import jax.numpy as jnp
from jax import lax
import jax.experimental.pallas as pl
import jax.experimental.pallas.tpu as pltpu

_NT = (((1,), (1,)), ((), ()))


def _layernorm(x, eps=1e-5):
    m = jnp.mean(x, axis=-1, keepdims=True)
    d = x - m
    v = jnp.mean(d * d, axis=-1, keepdims=True)
    return d / jnp.sqrt(v + eps)


def make(RB=512, L=2, pre=((0,), (1,)), mid=((2,), ()), G=16, DH=2, order=None, tail=((0, 1, 2, 3, 8, 9), (4, 5), (6,), (7,)),
         sem_checks=False, compute=True, unroll=1):
    def fn(A_x, A_k_cache, A_v_cache, A_wq, A_wo, B_x, B_w1, B_w2, B_w3, B_w4):
        B, Sq, D = A_x.shape
        _, H, Sk, Dh = A_k_cache.shape
        F = B_w3.shape[1]
        W = min(4096, max(256, Sk // 4))
        W0 = Sk - W
        HD = H * Dh
        scale = Dh ** -0.5
        f32, bf16 = jnp.float32, jnp.bfloat16
        NB = W // RB
        R = 128 // DH
        NG = H // G
        NU = B * NG
        ordr = order or tuple(range(G // DH))
        SR = 512
        PR = 32
        NSTEP = SR // PR
        NO = HD // SR
        NF = pl.cdiv(F, SR)
        FLAST = (F - (NF - 1) * SR) // PR
        assert L <= NB and len(pre) == L
        NSL = L + 1

        def kernel(x_hbm, k_hbm, v_hbm, wq_hbm, wo_hbm, w3t_hbm, w4_hbm, o_ref,
                   x_vm, wq_vm, wo_vm, w3_vm, w4_vm, buf, q_vm, s_vm, p_vm, a_vm,
                   wsem, bsem, osem):

            def loop(lo, hi, body, unroll=1):
                lax.fori_loop(lo, hi, lambda i, _: body(i), None, unroll=unroll)

            def wait_all(ref, sem):
                pltpu.make_async_copy(ref, ref, sem).wait()

            def issue_block(src, u, c, slot):
                b, h0 = u // NG, (u % NG) * G

                def body(i):
                    r = pl.multiple_of(i * R, R)
                    for e, j in enumerate(ordr):
                        pltpu.make_async_copy(
                            src.at[b, pl.ds(h0 + j * DH, DH), pl.ds(W0 + c * RB + r, R), :],
                            buf.at[slot, pl.ds(j * DH, DH), pl.ds(r, R), :],
                            bsem.at[slot]).start(priority=e % 2)
                loop(0, RB // R, body, unroll)

            def rows_piece(src, dst, sem, r):
                r = r if isinstance(r, int) else pl.multiple_of(r, PR)
                return pltpu.make_async_copy(src.at[pl.ds(r, PR), :], dst.at[pl.ds(r, PR), :], sem)

            def wq_piece(j, i):
                r = pl.multiple_of(j * (D // NO) + (i // 2) * 8, 8)
                c = pl.ds(pl.multiple_of((i % 2) * (HD // 2), HD // 2), HD // 2)
                return pltpu.make_async_copy(wq_hbm.at[pl.ds(r, 8), c], wq_vm.at[pl.ds(r, 8), c], wsem.at[1])

            xcp = pltpu.make_async_copy(x_hbm, x_vm, wsem.at[0])
            xcp.start()

            def phase_a(nf, par):
                def body(i):
                    cps = [wq_piece(j, i) for j in range(NO)]
                    cps += [rows_piece(w3t_hbm, w3_vm, wsem.at[2], j * SR + i * PR) for j in range(nf)]
                    for e, cp in enumerate(cps):
                        cp.start(priority=(e + par) % 2)
                return body

            def pairs(n):
                phase_a(NF, 0)(2 * n)
                phase_a(NF, 1)(2 * n + 1)
            loop(0, FLAST // 2, pairs)
            if FLAST % 2:
                phase_a(NF, 0)(jnp.int32(FLAST - 1))
            loop(FLAST, NSTEP, phase_a(NF - 1, 0))

            for c in range(L):
                issue_block(k_hbm, 0, c, c)
            xcp.wait()
            x = x_vm[...].astype(f32)
            xn = _layernorm(x).astype(bf16)
            xn2 = _layernorm(xn.astype(f32)).astype(bf16)
            wait_all(wq_vm, wsem.at[1])
            wait_all(w3_vm, wsem.at[2])
            if compute:
                for h in range(H):
                    q_vm[pl.ds(h, B, stride=H), :] = jnp.dot(
                        xn, wq_vm[:, h * Dh:(h + 1) * Dh], preferred_element_type=f32)

            def c_piece(j, i, sem):
                if j < NO:
                    return rows_piece(wo_hbm, wo_vm, sem, j * SR + i * PR)
                return rows_piece(w4_hbm, w4_vm, sem, (j - NO) * SR + i * PR)

            def c_streams(i):
                return range(NO + NF if i < FLAST else NO + NF - 1)

            per = Dh // PR
            groups = [[(j, i) for i in range(t * per, (t + 1) * per) for j in c_streams(i)]
                      for t in range(NSTEP // per - 1)]
            groups += [[(j, i) for i in range(NSTEP - per, NSTEP) for j in js] for js in tail]

            def issue_group(gi):
                for e, (j, i) in enumerate(groups[gi]):
                    c_piece(j, i, osem.at[gi]).start(priority=e % 2)

            row_s = lax.broadcasted_iota(jnp.int32, (8, RB), 0)
            row_o = lax.broadcasted_iota(jnp.int32, (8, Dh), 0)

            def unit(u):
                r0 = pl.multiple_of(u * G, G)

                def kstep(c):
                    n = 2 * NB * u + c
                    slot, nxt = lax.rem(n, NSL), lax.rem(n + L, NSL)

                    if L < NB:
                        @pl.when(c < NB - L)
                        def _():
                            issue_block(k_hbm, u, c + L, nxt)

                    @pl.when(c >= NB - L)
                    def _():
                        issue_block(v_hbm, u, c + L - NB, nxt)

                    wait_all(buf.at[slot], bsem.at[slot])
                    if not compute:
                        return
                    for g in range(G // 8):
                        q = q_vm[pl.ds(r0 + g * 8, 8), :].astype(bf16)
                        s = None
                        for j in range(8):
                            sj = lax.dot_general(q, buf[slot, g * 8 + j], _NT, preferred_element_type=f32)
                            s = sj if s is None else jnp.where(row_s == j, sj, s)
                        s_vm[c, pl.ds(g * 8, 8), :] = s * scale
                loop(0, NB, kstep)

                if compute:
                    m = jnp.max(s_vm[0], axis=-1, keepdims=True)
                    for c in range(1, NB):
                        m = jnp.maximum(m, jnp.max(s_vm[c], axis=-1, keepdims=True))
                    l = None
                    for c in range(NB):
                        p = jnp.exp(s_vm[c] - m)
                        p_vm[c] = p
                        l = p if l is None else l + p
                    l = jnp.sum(l, axis=-1, keepdims=True)

                def vstep(c, o):
                    n = 2 * NB * u + NB + c
                    slot, nxt = lax.rem(n, NSL), lax.rem(n + L, NSL)

                    if L < NB:
                        @pl.when(c < NB - L)
                        def _():
                            issue_block(v_hbm, u, c + L, nxt)

                    @pl.when(c >= NB - L)
                    def _():
                        @pl.when(u < NU - 1)
                        def _():
                            issue_block(k_hbm, u + 1, c + L - NB, nxt)

                        for t, gis in enumerate(pre):
                            if gis:
                                @pl.when(n == 2 * NB * NU - L + t)
                                def _():
                                    for gi in gis:
                                        issue_group(gi)

                    wait_all(buf.at[slot], bsem.at[slot])
                    if not compute:
                        return o
                    parts = []
                    for g in range(G // 8):
                        p = p_vm[c, pl.ds(g * 8, 8), :].astype(bf16)
                        t = None
                        for j in range(8):
                            tj = jnp.dot(p, buf[slot, g * 8 + j], preferred_element_type=f32)
                            t = tj if t is None else jnp.where(row_o == j, tj, t)
                        parts.append(t)
                    return o + jnp.concatenate(parts, axis=0)
                o = lax.fori_loop(0, NB, vstep, jnp.zeros((G, Dh), f32))
                if compute:
                    a_vm[pl.ds(r0, G), :] = o / l
            loop(0, NU, unit)

            acc = x + xn.astype(f32)
            for gi in mid[0]:
                issue_group(gi)
            if compute:
                g = lax.dot_general(xn2, w3_vm[...], _NT, preferred_element_type=f32)
                g = jax.nn.gelu(g, approximate=True).astype(bf16)
            for gi, grp in enumerate(groups):
                if gi + 1 < len(mid):
                    for gj in mid[gi + 1]:
                        issue_group(gj)
                if gi + 1 == len(mid):
                    for gj in range(len(groups)):
                        if not any(gj in t for t in pre + mid):
                            issue_group(gj)
                nrows = len(grp) * PR
                wait_all(wo_vm.at[pl.ds(0, nrows), :], osem.at[gi])
                if not compute:
                    continue
                for j in sorted({j for j, _ in grp}):
                    steps = [i for jj, i in grp if jj == j]
                    lo, n = min(steps) * PR, len(steps) * PR
                    if j < NO:
                        a = a_vm[pl.ds((j * SR + lo) // Dh, B, stride=H), :].astype(bf16)
                        w = wo_vm[pl.ds(j * SR + lo, n), :]
                    else:
                        r = (j - NO) * SR + lo
                        a = g[:, r:r + n]
                        w = w4_vm[pl.ds(r, n), :]
                    acc = acc + jnp.dot(a, w, preferred_element_type=f32)
            o_ref[...] = acc.astype(o_ref.dtype)

        ngroups = NSTEP // (Dh // PR) - 1 + len(tail)
        out = pl.pallas_call(
            kernel,
            in_specs=[pl.BlockSpec(memory_space=pltpu.HBM)] * 7,
            out_specs=pl.BlockSpec(memory_space=pltpu.VMEM),
            out_shape=jax.ShapeDtypeStruct((B, D), A_x.dtype),
            scratch_shapes=[
                pltpu.VMEM((B, D), bf16),
                pltpu.VMEM((D, HD), bf16),
                pltpu.VMEM((HD, D), bf16),
                pltpu.VMEM((F, D), bf16),
                pltpu.VMEM((F, D), bf16),
                pltpu.VMEM((NSL, G, RB, Dh), bf16),
                pltpu.VMEM((B * H, Dh), f32),
                pltpu.VMEM((NB, G, RB), f32),
                pltpu.VMEM((NB, G, RB), f32),
                pltpu.VMEM((B * H, Dh), f32),
                pltpu.SemaphoreType.DMA((3,)),
                pltpu.SemaphoreType.DMA((NSL,)),
                pltpu.SemaphoreType.DMA((ngroups,)),
            ],
            compiler_params=pltpu.CompilerParams(
                vmem_limit_bytes=64 * 1024 * 1024,
                disable_bounds_checks=True,
                disable_semaphore_checks=not sem_checks),
        )(A_x.reshape(B, D), A_k_cache, A_v_cache, A_wq, A_wo, B_w3.T, B_w4)
        return out.reshape(B, Sq, D)
    return fn


_impl = make(RB=512, L=2, pre=((0,),(1,)), mid=((2,),), tail=((0,1,2,3,4,5,8,9),(6,7)))


@jax.jit
def pallas_parallel_sum__sliding_block_cached__mixer_s_mlp__decode_kernel(
    A_x, A_k_cache, A_v_cache, A_wq, A_wo, B_x, B_w1, B_w2, B_w3, B_w4
):
    return _impl(A_x, A_k_cache, A_v_cache, A_wq, A_wo, B_x, B_w1, B_w2, B_w3, B_w4)
```

```python
import jax
import jax.numpy as jnp
from jax import lax
import jax.experimental.pallas as pl
import jax.experimental.pallas.tpu as pltpu

_NT = (((1,), (1,)), ((), ()))


def _layernorm(x, eps=1e-5):
    m = jnp.mean(x, axis=-1, keepdims=True)
    d = x - m
    v = jnp.mean(d * d, axis=-1, keepdims=True)
    return d / jnp.sqrt(v + eps)


def make(RB=256, L=4, DS=4, order=(0, 2, 1, 3, 4, 6, 5, 7), tail=(6, 2), compute=True, tail_at=1,
         mlp_first=True):
    def fn(A_x, A_k_cache, A_v_cache, A_wq, A_wo, B_x, B_w1, B_w2, B_w3, B_w4):
        B, Sq, D = A_x.shape
        _, H, Sk, Dh = A_k_cache.shape
        F = B_w3.shape[1]
        W = min(4096, max(256, Sk // 4))
        W0 = Sk - W
        HD = H * Dh
        scale = Dh ** -0.5
        f32, bf16 = jnp.float32, jnp.bfloat16
        G = 16
        NU = B * H // G
        NB = W // RB
        R = 64
        GH = G // (2 * DS)
        NSL = L + 1
        SR = 512
        PR = 32
        NSTEP = SR // PR
        NO = HD // SR
        NF = pl.cdiv(F, SR)
        FLAST = (F - (NF - 1) * SR) // PR
        PER = Dh // PR
        NT = NSTEP // PER
        assert L <= NB and sum(tail) == NO

        def kernel(x_hbm, k_hbm, v_hbm, wq_hbm, wo_hbm, w3t_hbm, w4_hbm, o_ref,
                   x_vm, wq_vm, wo_vm, w3_vm, w4_vm, buf, q_vm, s_vm, a_vm,
                   wsem, bsem, osem):

            def loop(lo, hi, body, unroll=1):
                lax.fori_loop(lo, hi, lambda i, _: body(i), None, unroll=unroll)

            def wait_all(ref, sem):
                pltpu.make_async_copy(ref, ref, sem).wait()

            def issue_block(src, u, c, slot):
                def body(i):
                    r = pl.multiple_of(i * R, R)
                    for e, j in enumerate(order):
                        hi, lo = divmod(j, DS)
                        pltpu.make_async_copy(
                            src.at[u * GH + hi, :, lo, pl.ds(W0 + c * RB + r, R), :],
                            buf.at[slot, hi, :, lo, pl.ds(r, R), :],
                            bsem.at[slot]).start(priority=e % 2)
                loop(0, RB // R, body)

            def rows_piece(src, dst, sem, r):
                r = r if isinstance(r, int) else pl.multiple_of(r, PR)
                return pltpu.make_async_copy(src.at[pl.ds(r, PR), :], dst.at[pl.ds(r, PR), :], sem)

            def mlp_steps(nf):
                def body(i):
                    for j in range(nf):
                        rows_piece(w3t_hbm, w3_vm, wsem.at[2], j * SR + i * PR).start(priority=0)
                        rows_piece(w4_hbm, w4_vm, wsem.at[2], j * SR + i * PR).start(priority=1)
                return body

            def wq_steps(i):
                r = pl.multiple_of(i * 8, 8)
                for half in range(2):
                    for j in range(NO):
                        idx = (pl.ds(j * (D // NO) + r, 8), pl.ds(half * (HD // 2), HD // 2))
                        pltpu.make_async_copy(wq_hbm.at[idx], wq_vm.at[idx], wsem.at[1]).start(priority=j % 2)

            xcp = pltpu.make_async_copy(x_hbm, x_vm, wsem.at[0])
            xcp.start()
            loop(0, FLAST, mlp_steps(NF))
            loop(FLAST, NSTEP, mlp_steps(NF - 1))
            loop(0, NSTEP // 2, wq_steps)

            xcp.wait()
            x = x_vm[...].astype(f32)
            xn = _layernorm(x).astype(bf16)
            xn2 = _layernorm(xn.astype(f32)).astype(bf16)
            acc = x + xn.astype(f32)
            wait_all(w3_vm, wsem.at[2])
            wait_all(w4_vm, wsem.at[2])

            def mlp(r, n, acc):
                g = lax.dot_general(xn2, w3_vm[pl.ds(r, n), :], _NT, preferred_element_type=f32)
                g = jax.nn.gelu(g, approximate=True).astype(bf16)
                return acc + jnp.dot(g, w4_vm[pl.ds(r, n), :], preferred_element_type=f32)

            FB = 256
            if compute:
                acc = lax.fori_loop(0, F // FB, lambda i, a: mlp(pl.multiple_of(i * FB, FB), FB, a), acc)
                if F % FB:
                    acc = mlp(F // FB * FB, F % FB, acc)

            loop(0, L, lambda c: issue_block(k_hbm, 0, c, c))
            wait_all(wq_vm, wsem.at[1])

            QB = 512

            def qproj(i):
                q = jnp.dot(xn, wq_vm[:, pl.ds(pl.multiple_of(i * QB, QB), QB)], preferred_element_type=f32)
                for t in range(QB // Dh):
                    q_vm[pl.ds(i * (QB // Dh) + t, B, stride=H), :] = q[:, t * Dh:(t + 1) * Dh]
            if compute:
                loop(0, HD // QB, qproj)

            def wo_steps(lo, hi, js, sem):
                def body(i):
                    for e, j in enumerate(js):
                        rows_piece(wo_hbm, wo_vm, sem, j * SR + i * PR).start(priority=e % 2)
                loop(lo, hi, body)

            row_s = lax.broadcasted_iota(jnp.int32, (8, RB), 0)
            row_o = lax.broadcasted_iota(jnp.int32, (8, Dh), 0)

            def head(slot, g, j):
                hi, rest = divmod(j, 2 * DS)
                return buf[slot, g * (8 // (2 * DS)) + hi, rest // DS, rest % DS]

            def unit(u):
                r0 = u * G

                def kstep(c):
                    n = 2 * NB * u + c
                    slot, nxt = lax.rem(n, NSL), lax.rem(n + L, NSL)

                    if L < NB:
                        @pl.when(c < NB - L)
                        def _():
                            issue_block(k_hbm, u, c + L, nxt)

                    @pl.when(c >= NB - L)
                    def _():
                        issue_block(v_hbm, u, c + L - NB, nxt)

                    wait_all(buf.at[slot], bsem.at[slot])

                    def half(g):
                        q = q_vm[pl.ds(pl.multiple_of(r0 + g * 8, 8), 8), :].astype(bf16)
                        s = None
                        for j in range(8):
                            sj = lax.dot_general(q, head(slot, g, j), _NT, preferred_element_type=f32)
                            s = sj if s is None else jnp.where(row_s == j, sj, s)
                        s_vm[c, g] = s * scale
                    if compute:
                        loop(0, G // 8, half)
                loop(0, NB, kstep)

                def softmax(g):
                    s = [s_vm[c, g] for c in range(NB)]
                    m = s[0]
                    for c in range(1, NB):
                        m = jnp.maximum(m, s[c])
                    m = jnp.max(m, axis=-1, keepdims=True)
                    p = [jnp.exp(t - m) for t in s]
                    l = p[0]
                    for c in range(1, NB):
                        l = l + p[c]
                    inv = 1.0 / jnp.sum(l, axis=-1, keepdims=True)
                    for c in range(NB):
                        s_vm[c, g] = p[c] * inv
                    a_vm[pl.ds(pl.multiple_of(r0 + g * 8, 8), 8), :] = jnp.zeros((8, Dh), f32)
                if compute:
                    loop(0, G // 8, softmax)

                def vstep(c):
                    n = 2 * NB * u + NB + c
                    slot, nxt = lax.rem(n, NSL), lax.rem(n + L, NSL)

                    if L < NB:
                        @pl.when(c < NB - L)
                        def _():
                            issue_block(v_hbm, u, c + L, nxt)

                    @pl.when(c >= NB - L)
                    def _():
                        t = c + L - NB

                        @pl.when(u < NU - 1)
                        def _():
                            issue_block(k_hbm, u + 1, t, nxt)

                        @pl.when(u == NU - 1)
                        def _():
                            @pl.when(t < NT - 1)
                            def _():
                                wo_steps(t * PER, (t + 1) * PER, range(NO), osem.at[t])

                    wait_all(buf.at[slot], bsem.at[slot])

                    def half(g):
                        p = s_vm[c, g].astype(bf16)
                        t = None
                        for j in range(8):
                            tj = jnp.dot(p, head(slot, g, j), preferred_element_type=f32)
                            t = tj if t is None else jnp.where(row_o == j, tj, t)
                        a_vm[pl.ds(pl.multiple_of(r0 + g * 8, 8), 8), :] += t
                    if compute:
                        loop(0, G // 8, half)
                loop(0, NB, vstep)
            loop(0, NU, unit)

            for t in range(L, NT - 1):
                wo_steps(t * PER, (t + 1) * PER, range(NO), osem.at[t])

            def oproj(t, js, sem, acc):
                wait_all(wo_vm.at[pl.ds(0, len(js) * Dh), :], sem)
                if not compute:
                    return acc
                for j in js:
                    h = j * NT + t
                    a = a_vm[pl.ds(h, B, stride=H), :].astype(bf16)
                    r = h * Dh if isinstance(h, int) else pl.multiple_of(h * Dh, Dh)
                    acc = acc + jnp.dot(a, wo_vm[pl.ds(r, Dh), :], preferred_element_type=f32)
                return acc

            tails = [range(sum(tail[:i]), sum(tail[:i + 1])) for i in range(len(tail))]

            def ostep(t, acc):
                @pl.when(t == tail_at)
                def _():
                    for gi, js in enumerate(tails):
                        if len(js) % 2 == 0:
                            wo_steps(NSTEP - PER, NSTEP, js, osem.at[NT - 1 + gi])
                        else:
                            for e, (i, j) in enumerate((i, j) for i in range(NSTEP - PER, NSTEP) for j in js):
                                rows_piece(wo_hbm, wo_vm, osem.at[NT - 1 + gi], j * SR + i * PR).start(priority=e % 2)
                return oproj(t, range(NO), osem.at[t], acc)
            acc = lax.fori_loop(0, NT - 1, ostep, acc)
            for gi, js in enumerate(tails):
                acc = oproj(NT - 1, js, osem.at[NT - 1 + gi], acc)
            o_ref[...] = acc.astype(o_ref.dtype)

        kv_shape = (B * H // (2 * DS), 2, DS, Sk, Dh)
        out = pl.pallas_call(
            kernel,
            in_specs=[pl.BlockSpec(memory_space=pltpu.HBM)] * 7,
            out_specs=pl.BlockSpec(memory_space=pltpu.VMEM),
            out_shape=jax.ShapeDtypeStruct((B, D), A_x.dtype),
            scratch_shapes=[
                pltpu.VMEM((B, D), bf16),
                pltpu.VMEM((D, HD), bf16),
                pltpu.VMEM((HD, D), bf16),
                pltpu.VMEM((F, D), bf16),
                pltpu.VMEM((F, D), bf16),
                pltpu.VMEM((NSL, GH, 2, DS, RB, Dh), bf16),
                pltpu.VMEM((B * H, Dh), f32),
                pltpu.VMEM((NB, G // 8, 8, RB), f32),
                pltpu.VMEM((B * H, Dh), f32),
                pltpu.SemaphoreType.DMA((3,)),
                pltpu.SemaphoreType.DMA((NSL,)),
                pltpu.SemaphoreType.DMA((NT - 1 + len(tail),)),
            ],
            compiler_params=pltpu.CompilerParams(
                vmem_limit_bytes=64 * 1024 * 1024,
                disable_bounds_checks=True,
                disable_semaphore_checks=True),
        )(A_x.reshape(B, D), A_k_cache.reshape(kv_shape), A_v_cache.reshape(kv_shape),
          A_wq, A_wo, B_w3.T, B_w4)
        return out.reshape(B, Sq, D)
    return fn


_impl = make(tail=(4,2,2))


@jax.jit
def pallas_parallel_sum__sliding_block_cached__mixer_s_mlp__decode_kernel(
    A_x, A_k_cache, A_v_cache, A_wq, A_wo, B_x, B_w1, B_w2, B_w3, B_w4
):
    return _impl(A_x, A_k_cache, A_v_cache, A_wq, A_wo, B_x, B_w1, B_w2, B_w3, B_w4)
```

```python
import jax
import jax.numpy as jnp
from jax import lax
import jax.experimental.pallas as pl
import jax.experimental.pallas.tpu as pltpu

_NT = (((1,), (1,)), ((), ()))

_UNIT = 16
_HEAD_STRIDE = 4
_KV_ROWS = 64
_KV_ORDER = (0, 2, 1, 3, 4, 6, 5, 7)
_KV_BLOCK = 256
_AHEAD = 4
_W_ROWS = 32
_W_STREAM = 512
_MLP_BLOCK = 256
_Q_BLOCK = 512
_WO_TAIL = (4, 2, 2)


def _layernorm(x, eps=1e-5):
    d = x - jnp.mean(x, axis=-1, keepdims=True)
    var = jnp.mean(d * d, axis=-1, keepdims=True)
    return d / jnp.sqrt(var + eps)


def _loop(lo, hi, body):
    lax.fori_loop(lo, hi, lambda i, _: body(i), None)


def _wait_filled(ref, sem):
    pltpu.make_async_copy(ref, ref, sem).wait()


@jax.jit
def pallas_parallel_sum__sliding_block_cached__mixer_s_mlp__decode_kernel(
    A_x: jax.Array,
    A_k_cache: jax.Array,
    A_v_cache: jax.Array,
    A_wq: jax.Array,
    A_wo: jax.Array,
    B_x: jax.Array,
    B_w1: jax.Array,
    B_w2: jax.Array,
    B_w3: jax.Array,
    B_w4: jax.Array,
):
    B, S, D = A_x.shape
    _, H, Sk, Dh = A_k_cache.shape
    HD, F = H * Dh, B_w3.shape[1]
    W = min(4096, max(256, Sk // 4))
    f32, bf16 = jnp.float32, jnp.bfloat16

    assert S == 1 and A_wq.shape == (D, HD)
    del B_x, B_w1, B_w2

    n_units = B * H // _UNIT
    n_blocks = W // _KV_BLOCK
    n_slots = _AHEAD + 1
    n_steps = _W_STREAM // _W_ROWS
    n_wo = HD // _W_STREAM
    n_mlp = pl.cdiv(F, _W_STREAM)
    mlp_last = (F - (n_mlp - 1) * _W_STREAM) // _W_ROWS
    n_tiles = _W_STREAM // Dh
    tails = [(sum(_WO_TAIL[:i]), n) for i, n in enumerate(_WO_TAIL)]
    assert B < 8 and H % _UNIT == 0 and W % _KV_BLOCK == 0 and F % _W_ROWS == 0
    assert sum(_WO_TAIL) == n_wo and n_tiles - 1 <= _AHEAD <= n_blocks

    def kernel(x_hbm, k_hbm, v_hbm, wq_hbm, wo_hbm, w3t_hbm, w4_hbm, o_ref,
               x_vm, wq_vm, wo_vm, w3t_vm, w4_vm, kv_vm, q_vm, s_vm, a_vm,
               w_sem, kv_sem, wo_sem):

        def fetch_mlp(streams):
            def step(i):
                for j in range(streams):
                    rows = pl.ds(pl.multiple_of(j * _W_STREAM + i * _W_ROWS, _W_ROWS), _W_ROWS)
                    pltpu.make_async_copy(
                        w3t_hbm.at[rows], w3t_vm.at[rows], w_sem.at[2]).start(priority=0)
                    pltpu.make_async_copy(
                        w4_hbm.at[rows], w4_vm.at[rows], w_sem.at[3]).start(priority=1)
            return step

        def fetch_wq(i):
            for half in range(2):
                for j in range(n_wo):
                    idx = (pl.ds(pl.multiple_of(j * (D // n_wo) + i * 8, 8), 8),
                           pl.ds(half * (HD // 2), HD // 2))
                    pltpu.make_async_copy(
                        wq_hbm.at[idx], wq_vm.at[idx], w_sem.at[1]).start(priority=j % 2)

        def fetch_kv(src, unit, block, slot):
            def step(i):
                r = pl.multiple_of(i * _KV_ROWS, _KV_ROWS)
                for n, j in enumerate(_KV_ORDER):
                    g, lo = divmod(j, _HEAD_STRIDE)
                    pltpu.make_async_copy(
                        src.at[unit * (_UNIT // 8) + g, :, lo,
                               pl.ds(Sk - W + block * _KV_BLOCK + r, _KV_ROWS), :],
                        kv_vm.at[slot, g, :, lo, pl.ds(r, _KV_ROWS), :],
                        kv_sem.at[slot]).start(priority=n % 2)
            _loop(0, _KV_BLOCK // _KV_ROWS, step)

        def fetch_wo(tile, first, count, sem):
            def step(i):
                rows = pl.ds(pl.multiple_of(i * _W_ROWS, _W_ROWS), _W_ROWS)
                for n in range(count):
                    pltpu.make_async_copy(
                        wo_hbm.at[first + n, tile, rows, :], wo_vm.at[first + n, tile, rows, :],
                        sem).start(priority=n % 2)
            _loop(0, Dh // _W_ROWS, step)

        x_copy = pltpu.make_async_copy(x_hbm, x_vm, w_sem.at[0])
        x_copy.start()
        _loop(0, mlp_last, fetch_mlp(n_mlp))
        _loop(mlp_last, n_steps, fetch_mlp(n_mlp - 1))
        _loop(0, D // n_wo // 8, fetch_wq)

        x_copy.wait()
        x = x_vm[...].astype(f32)
        xn = _layernorm(x).astype(bf16)
        xn2 = _layernorm(xn.astype(f32)).astype(bf16)
        _wait_filled(w3t_vm, w_sem.at[2])
        _wait_filled(w4_vm, w_sem.at[3])

        def mlp(rows, acc):
            h = lax.dot_general(xn2, w3t_vm[rows, :], _NT, preferred_element_type=f32)
            h = jax.nn.gelu(h, approximate=True).astype(bf16)
            return acc + jnp.dot(h, w4_vm[rows, :], preferred_element_type=f32)

        acc = lax.fori_loop(
            0, F // _MLP_BLOCK,
            lambda i, acc: mlp(pl.ds(pl.multiple_of(i * _MLP_BLOCK, _MLP_BLOCK), _MLP_BLOCK), acc),
            x + xn.astype(f32))
        if F % _MLP_BLOCK:
            acc = mlp(pl.ds(F - F % _MLP_BLOCK, F % _MLP_BLOCK), acc)

        _loop(0, _AHEAD, lambda c: fetch_kv(k_hbm, 0, c, c))
        _wait_filled(wq_vm, w_sem.at[1])

        def project_q(i):
            cols = pl.ds(pl.multiple_of(i * _Q_BLOCK, _Q_BLOCK), _Q_BLOCK)
            q = jnp.dot(xn, wq_vm[:, cols], preferred_element_type=f32)
            for t in range(_Q_BLOCK // Dh):
                q_vm[pl.ds(i * (_Q_BLOCK // Dh) + t, B, stride=H), :] = q[:, t * Dh:(t + 1) * Dh]
        _loop(0, HD // _Q_BLOCK, project_q)

        def per_head(slot, g, matmul):
            out = None
            for j in range(8):
                y = matmul(kv_vm[slot, g, j // _HEAD_STRIDE, j % _HEAD_STRIDE])
                row = lax.broadcasted_iota(jnp.int32, y.shape, 0)
                out = y if out is None else jnp.where(row == j, y, out)
            return out

        def attend(unit):
            def heads(g):
                return pl.ds(pl.multiple_of(unit * _UNIT + g * 8, 8), 8)

            def scores(c):
                n = 2 * n_blocks * unit + c
                slot, free = lax.rem(n, n_slots), lax.rem(n + _AHEAD, n_slots)

                @pl.when(c + _AHEAD < n_blocks)
                def _():
                    fetch_kv(k_hbm, unit, c + _AHEAD, free)

                @pl.when(c + _AHEAD >= n_blocks)
                def _():
                    fetch_kv(v_hbm, unit, c + _AHEAD - n_blocks, free)

                _wait_filled(kv_vm.at[slot], kv_sem.at[slot])

                def group(g):
                    q = q_vm[heads(g), :].astype(bf16)
                    s_vm[c, g] = Dh ** -0.5 * per_head(
                        slot, g, lambda k: lax.dot_general(q, k, _NT, preferred_element_type=f32))
                _loop(0, _UNIT // 8, group)
            _loop(0, n_blocks, scores)

            def softmax(g):
                s = [s_vm[c, g] for c in range(n_blocks)]
                m = s[0]
                for t in s[1:]:
                    m = jnp.maximum(m, t)
                m = jnp.max(m, axis=-1, keepdims=True)
                p = [jnp.exp(t - m) for t in s]
                inv = 1.0 / jnp.sum(sum(p[1:], p[0]), axis=-1, keepdims=True)
                for c in range(n_blocks):
                    s_vm[c, g] = p[c] * inv
                a_vm[heads(g), :] = jnp.zeros((8, Dh), f32)
            _loop(0, _UNIT // 8, softmax)

            def values(c):
                n = 2 * n_blocks * unit + n_blocks + c
                slot, free = lax.rem(n, n_slots), lax.rem(n + _AHEAD, n_slots)
                nxt = c + _AHEAD - n_blocks

                @pl.when(nxt < 0)
                def _():
                    fetch_kv(v_hbm, unit, c + _AHEAD, free)

                @pl.when(nxt >= 0)
                def _():
                    @pl.when(unit < n_units - 1)
                    def _():
                        fetch_kv(k_hbm, unit + 1, nxt, free)

                    @pl.when(jnp.logical_and(unit == n_units - 1, nxt < n_tiles - 1))
                    def _():
                        fetch_wo(nxt, 0, n_wo, wo_sem.at[nxt])

                _wait_filled(kv_vm.at[slot], kv_sem.at[slot])

                def group(g):
                    p = s_vm[c, g].astype(bf16)
                    a_vm[heads(g), :] += per_head(
                        slot, g, lambda v: jnp.dot(p, v, preferred_element_type=f32))
                _loop(0, _UNIT // 8, group)
            _loop(0, n_blocks, values)
        _loop(0, n_units, attend)

        def pad_rows(y):
            return jnp.concatenate([y, jnp.zeros((8 - B, y.shape[1]), f32)], axis=0)

        def project_out(tile, first, count, sem, acc):
            a = [pad_rows(a_vm[pl.ds(j * n_tiles + tile, B, stride=H), :]).astype(bf16)
                 for j in range(first, first + count)]
            _wait_filled(wo_vm.at[pl.ds(first, count), tile], sem)
            for n in range(count):
                acc = acc + jnp.dot(a[n], wo_vm[first + n, tile], preferred_element_type=f32)
            return acc

        def out_step(tile, acc):
            @pl.when(tile == 1)
            def _():
                for i, (first, count) in enumerate(tails):
                    fetch_wo(n_tiles - 1, first, count, wo_sem.at[n_tiles - 1 + i])
            return project_out(tile, 0, n_wo, wo_sem.at[tile], acc)

        acc = lax.fori_loop(0, n_tiles - 1, out_step, pad_rows(acc))
        for i, (first, count) in enumerate(tails):
            acc = project_out(n_tiles - 1, first, count, wo_sem.at[n_tiles - 1 + i], acc)
        o_ref[...] = acc[:B].astype(o_ref.dtype)

    kv_shape = (B * H // 8, 8 // _HEAD_STRIDE, _HEAD_STRIDE, Sk, Dh)
    out = pl.pallas_call(
        kernel,
        in_specs=[pl.BlockSpec(memory_space=pltpu.HBM)] * 7,
        out_specs=pl.BlockSpec(memory_space=pltpu.VMEM),
        out_shape=jax.ShapeDtypeStruct((B, D), A_x.dtype),
        scratch_shapes=[
            pltpu.VMEM((B, D), bf16),
            pltpu.VMEM((D, HD), bf16),
            pltpu.VMEM((n_wo, n_tiles, Dh, D), bf16),
            pltpu.VMEM((F, D), bf16),
            pltpu.VMEM((F, D), bf16),
            pltpu.VMEM((n_slots, _UNIT // 8) + kv_shape[1:3] + (_KV_BLOCK, Dh), bf16),
            pltpu.VMEM(((B + 1) * H, Dh), f32),
            pltpu.VMEM((n_blocks, _UNIT // 8, 8, _KV_BLOCK), f32),
            pltpu.VMEM(((B + 1) * H, Dh), f32),
            pltpu.SemaphoreType.DMA((4,)),
            pltpu.SemaphoreType.DMA((n_slots,)),
            pltpu.SemaphoreType.DMA((n_tiles - 1 + len(tails),)),
        ],
        compiler_params=pltpu.CompilerParams(
            vmem_limit_bytes=48 * 1024 * 1024,
            disable_semaphore_checks=True),
    )(A_x.reshape(B, D), A_k_cache.reshape(kv_shape), A_v_cache.reshape(kv_shape),
      A_wq, A_wo.reshape(n_wo, n_tiles, Dh, D), B_w3.T, B_w4)
    return out.reshape(B, S, D)
```

```python
import jax
import jax.numpy as jnp
from jax import lax
import jax.experimental.pallas as pl
import jax.experimental.pallas.tpu as pltpu

_NT = (((1,), (1,)), ((), ()))

_UNIT = 16
_HEAD_STRIDE = 4
_KV_ROWS = 64
_KV_ORDER = (0, 2, 1, 3, 4, 6, 5, 7)
_KV_BLOCK = 256
_AHEAD = 4
_W_ROWS = 32
_W_STREAM = 512
_MLP_BLOCK = 256
_Q_BLOCK = 512
_WO_TAIL = (4, 2, 2)


def _layernorm(x, eps=1e-5):
    d = x - jnp.mean(x, axis=-1, keepdims=True)
    var = jnp.mean(d * d, axis=-1, keepdims=True)
    return d / jnp.sqrt(var + eps)


def _loop(lo, hi, body):
    lax.fori_loop(lo, hi, lambda i, _: body(i), None)


def _wait_filled(ref, sem):
    pltpu.make_async_copy(ref, ref, sem).wait()


@jax.jit
def pallas_parallel_sum__sliding_block_cached__mixer_s_mlp__decode_kernel(
    A_x: jax.Array,
    A_k_cache: jax.Array,
    A_v_cache: jax.Array,
    A_wq: jax.Array,
    A_wo: jax.Array,
    B_x: jax.Array,
    B_w1: jax.Array,
    B_w2: jax.Array,
    B_w3: jax.Array,
    B_w4: jax.Array,
):
    B, S, D = A_x.shape
    _, H, Sk, Dh = A_k_cache.shape
    HD, F = H * Dh, B_w3.shape[1]
    W = min(4096, max(256, Sk // 4))
    f32, bf16 = jnp.float32, jnp.bfloat16

    assert S == 1 and A_wq.shape == (D, HD)
    del B_x, B_w1, B_w2

    n_units = B * H // _UNIT
    n_blocks = W // _KV_BLOCK
    n_slots = _AHEAD + 1
    n_steps = _W_STREAM // _W_ROWS
    n_wo = HD // _W_STREAM
    n_mlp = pl.cdiv(F, _W_STREAM)
    mlp_last = (F - (n_mlp - 1) * _W_STREAM) // _W_ROWS
    n_tiles = _W_STREAM // Dh
    tails = [(sum(_WO_TAIL[:i]), n) for i, n in enumerate(_WO_TAIL)]
    assert B < 8 and H % _UNIT == 0 and W % _KV_BLOCK == 0 and F % _W_ROWS == 0
    assert sum(_WO_TAIL) == n_wo and n_tiles - 1 <= _AHEAD <= n_blocks

    def kernel(x_hbm, k_hbm, v_hbm, wq_hbm, wo_hbm, w3t_hbm, w4_hbm, o_ref,
               x_vm, wq_vm, wo_vm, w3t_vm, w4_vm, kv_vm, q_vm, s_vm, a_vm,
               w_sem, kv_sem, wo_sem):

        def fetch_mlp(streams):
            def step(i):
                for j in range(streams):
                    rows = pl.ds(pl.multiple_of(j * _W_STREAM + i * _W_ROWS, _W_ROWS), _W_ROWS)
                    pltpu.make_async_copy(
                        w3t_hbm.at[rows], w3t_vm.at[rows], w_sem.at[2]).start(priority=0)
                    pltpu.make_async_copy(
                        w4_hbm.at[rows], w4_vm.at[rows], w_sem.at[3]).start(priority=1)
            return step

        def fetch_wq(i):
            for half in range(2):
                for j in range(n_wo):
                    idx = (j * (D // 8 // n_wo) + i, slice(None), pl.ds(half * (HD // 2), HD // 2))
                    pltpu.make_async_copy(
                        wq_hbm.at[idx], wq_vm.at[idx], w_sem.at[1]).start(priority=j % 2)

        def fetch_kv(src, unit, block, slot):
            def step(i):
                r = pl.multiple_of(i * _KV_ROWS, _KV_ROWS)
                for n, j in enumerate(_KV_ORDER):
                    g, lo = divmod(j, _HEAD_STRIDE)
                    pltpu.make_async_copy(
                        src.at[unit * (_UNIT // 8) + g, :, lo,
                               pl.ds(Sk - W + block * _KV_BLOCK + r, _KV_ROWS), :],
                        kv_vm.at[slot, g, :, lo, pl.ds(r, _KV_ROWS), :],
                        kv_sem.at[slot]).start(priority=n % 2)
            _loop(0, _KV_BLOCK // _KV_ROWS, step)

        def fetch_wo(tile, first, count, sem):
            def step(i):
                rows = pl.ds(pl.multiple_of(i * _W_ROWS, _W_ROWS), _W_ROWS)
                for n in range(count):
                    pltpu.make_async_copy(
                        wo_hbm.at[first + n, tile, rows, :], wo_vm.at[first + n, tile, rows, :],
                        sem).start(priority=n % 2)
            _loop(0, Dh // _W_ROWS, step)

        x_copy = pltpu.make_async_copy(x_hbm, x_vm, w_sem.at[0])
        x_copy.start()
        _loop(0, mlp_last, fetch_mlp(n_mlp))
        _loop(mlp_last, n_steps, fetch_mlp(n_mlp - 1))
        _loop(0, D // 8 // n_wo, fetch_wq)

        x_copy.wait()
        x = x_vm[...].astype(f32)
        xn = _layernorm(x).astype(bf16)
        xn2 = _layernorm(xn.astype(f32)).astype(bf16)
        _wait_filled(w3t_vm, w_sem.at[2])
        _wait_filled(w4_vm, w_sem.at[3])

        def mlp(rows, acc):
            h = lax.dot_general(xn2, w3t_vm[rows, :], _NT, preferred_element_type=f32)
            h = jax.nn.gelu(h, approximate=True).astype(bf16)
            return acc + jnp.dot(h, w4_vm[rows, :], preferred_element_type=f32)

        acc = lax.fori_loop(
            0, F // _MLP_BLOCK,
            lambda i, acc: mlp(pl.ds(pl.multiple_of(i * _MLP_BLOCK, _MLP_BLOCK), _MLP_BLOCK), acc),
            x + xn.astype(f32))
        if F % _MLP_BLOCK:
            acc = mlp(pl.ds(F - F % _MLP_BLOCK, F % _MLP_BLOCK), acc)

        _loop(0, _AHEAD, lambda c: fetch_kv(k_hbm, 0, c, c))
        _wait_filled(wq_vm, w_sem.at[1])

        def project_q(i):
            cols = pl.ds(pl.multiple_of(i * _Q_BLOCK, _Q_BLOCK), _Q_BLOCK)
            q = jnp.dot(xn, wq_vm[:, :, cols].reshape(D, _Q_BLOCK), preferred_element_type=f32)
            for t in range(_Q_BLOCK // Dh):
                q_vm[pl.ds(i * (_Q_BLOCK // Dh) + t, B, stride=H), :] = q[:, t * Dh:(t + 1) * Dh]
        _loop(0, HD // _Q_BLOCK, project_q)

        def per_head(slot, g, matmul):
            out = None
            for j in range(8):
                y = matmul(kv_vm[slot, g, j // _HEAD_STRIDE, j % _HEAD_STRIDE])
                row = lax.broadcasted_iota(jnp.int32, y.shape, 0)
                out = y if out is None else jnp.where(row == j, y, out)
            return out

        def attend(unit):
            def heads(g):
                return pl.ds(pl.multiple_of(unit * _UNIT + g * 8, 8), 8)

            def scores(c):
                n = 2 * n_blocks * unit + c
                slot, free = lax.rem(n, n_slots), lax.rem(n + _AHEAD, n_slots)

                @pl.when(c + _AHEAD < n_blocks)
                def _():
                    fetch_kv(k_hbm, unit, c + _AHEAD, free)

                @pl.when(c + _AHEAD >= n_blocks)
                def _():
                    fetch_kv(v_hbm, unit, c + _AHEAD - n_blocks, free)

                _wait_filled(kv_vm.at[slot], kv_sem.at[slot])

                def group(g):
                    q = q_vm[heads(g), :].astype(bf16)
                    s_vm[c, g] = Dh ** -0.5 * per_head(
                        slot, g, lambda k: lax.dot_general(q, k, _NT, preferred_element_type=f32))
                _loop(0, _UNIT // 8, group)
            _loop(0, n_blocks, scores)

            def softmax(g):
                s = [s_vm[c, g] for c in range(n_blocks)]
                m = s[0]
                for t in s[1:]:
                    m = jnp.maximum(m, t)
                m = jnp.max(m, axis=-1, keepdims=True)
                p = [jnp.exp(t - m) for t in s]
                inv = 1.0 / jnp.sum(sum(p[1:], p[0]), axis=-1, keepdims=True)
                for c in range(n_blocks):
                    s_vm[c, g] = p[c] * inv
                a_vm[heads(g), :] = jnp.zeros((8, Dh), f32)
            _loop(0, _UNIT // 8, softmax)

            def values(c):
                n = 2 * n_blocks * unit + n_blocks + c
                slot, free = lax.rem(n, n_slots), lax.rem(n + _AHEAD, n_slots)
                nxt = c + _AHEAD - n_blocks

                @pl.when(nxt < 0)
                def _():
                    fetch_kv(v_hbm, unit, c + _AHEAD, free)

                @pl.when(nxt >= 0)
                def _():
                    @pl.when(unit < n_units - 1)
                    def _():
                        fetch_kv(k_hbm, unit + 1, nxt, free)

                    @pl.when(jnp.logical_and(unit == n_units - 1, nxt < n_tiles - 1))
                    def _():
                        fetch_wo(nxt, 0, n_wo, wo_sem.at[nxt])

                _wait_filled(kv_vm.at[slot], kv_sem.at[slot])

                def group(g):
                    p = s_vm[c, g].astype(bf16)
                    a_vm[heads(g), :] += per_head(
                        slot, g, lambda v: jnp.dot(p, v, preferred_element_type=f32))
                _loop(0, _UNIT // 8, group)
            _loop(0, n_blocks, values)
        _loop(0, n_units, attend)

        def pad_rows(y):
            return jnp.concatenate([y, jnp.zeros((8 - B, y.shape[1]), f32)], axis=0)

        def project_out(tile, first, count, sem, acc):
            a = [pad_rows(a_vm[pl.ds(j * n_tiles + tile, B, stride=H), :]).astype(bf16)
                 for j in range(first, first + count)]
            _wait_filled(wo_vm.at[pl.ds(first, count), tile], sem)
            for n in range(count):
                acc = acc + jnp.dot(a[n], wo_vm[first + n, tile], preferred_element_type=f32)
            return acc

        def out_step(tile, acc):
            @pl.when(tile == 1)
            def _():
                for i, (first, count) in enumerate(tails):
                    fetch_wo(n_tiles - 1, first, count, wo_sem.at[n_tiles - 1 + i])
            return project_out(tile, 0, n_wo, wo_sem.at[tile], acc)

        acc = lax.fori_loop(0, n_tiles - 1, out_step, pad_rows(acc))
        for i, (first, count) in enumerate(tails):
            acc = project_out(n_tiles - 1, first, count, wo_sem.at[n_tiles - 1 + i], acc)
        o_ref[...] = acc[:B].astype(o_ref.dtype)

    kv_shape = (B * H // 8, 8 // _HEAD_STRIDE, _HEAD_STRIDE, Sk, Dh)
    out = pl.pallas_call(
        kernel,
        in_specs=[pl.BlockSpec(memory_space=pltpu.HBM)] * 7,
        out_specs=pl.BlockSpec(memory_space=pltpu.VMEM),
        out_shape=jax.ShapeDtypeStruct((B, D), A_x.dtype),
        scratch_shapes=[
            pltpu.VMEM((B, D), bf16),
            pltpu.VMEM((D // 8, 8, HD), bf16),
            pltpu.VMEM((n_wo, n_tiles, Dh, D), bf16),
            pltpu.VMEM((F, D), bf16),
            pltpu.VMEM((F, D), bf16),
            pltpu.VMEM((n_slots, _UNIT // 8) + kv_shape[1:3] + (_KV_BLOCK, Dh), bf16),
            pltpu.VMEM(((B + 1) * H, Dh), f32),
            pltpu.VMEM((n_blocks, _UNIT // 8, 8, _KV_BLOCK), f32),
            pltpu.VMEM(((B + 1) * H, Dh), f32),
            pltpu.SemaphoreType.DMA((4,)),
            pltpu.SemaphoreType.DMA((n_slots,)),
            pltpu.SemaphoreType.DMA((n_tiles - 1 + len(tails),)),
        ],
        compiler_params=pltpu.CompilerParams(
            vmem_limit_bytes=48 * 1024 * 1024,
            disable_semaphore_checks=True),
    )(A_x.reshape(B, D), A_k_cache.reshape(kv_shape), A_v_cache.reshape(kv_shape),
      A_wq.reshape(D // 8, 8, HD), A_wo.reshape(n_wo, n_tiles, Dh, D), B_w3.T, B_w4)
    return out.reshape(B, S, D)
```
